```python
import jax
import jax.numpy as jnp

def _softmax(x, axis=-1):
    return jax.nn.softmax(x, axis=axis)
def _gelu(x):
    return jax.nn.gelu(x, approximate=True)
def _silu(x):
    return jax.nn.silu(x)
def _sigmoid(x):
    return jax.nn.sigmoid(x)
def _layernorm(x, axis=-1, eps=1e-5):
    m = jnp.mean(x, axis=axis, keepdims=True)
    v = jnp.var(x, axis=axis, keepdims=True)
    return (x - m) / jnp.sqrt(v + eps)
def _scatter_add(tgt, idx, src, axis=0):
    return tgt.at[idx].add(src)
def _segment_sum(src, seg, n):
    return jax.ops.segment_sum(src, seg, n)
class _Rng:
    def __init__(self, key):
        self._k = key
    def _next(self):
        self._k, sub = jax.random.split(self._k)
        return sub
    def normal(self, shape):
        return jax.random.normal(self._next(), shape, dtype=jnp.bfloat16)
    def randint(self, lo, hi, shape):
        return jax.random.randint(self._next(), shape, lo, hi, dtype=jnp.int32)
    def uniform(self, shape, lo=0.0, hi=1.0):
        return jax.random.uniform(self._next(), shape, jnp.bfloat16, lo, hi)
    def permutation(self, n):
        return jax.random.permutation(self._next(), n)


kernel_name = 'concat_heads__compressed_kv_cla__mha_block_cached__decode'

def setup_inputs():
    _rng = _Rng(jax.random.key(int.from_bytes(__import__("os").urandom(4), "little")))
    _w = (lambda a: (lambda t: t.astype(jnp.bfloat16) if jnp.issubdtype(t.dtype, jnp.floating) else t)(jnp.asarray(a)))
    def _A_setup():
        B, H, Sq, Sk, D, M = 4, 32, 1, 4096, 128, 512
        Dc = 4 * D
        return {
            "x": _w((lambda *s: _rng.normal(s) * 0.05)(B, Sq, M)),
            "c_kv": _w((lambda *s: _rng.normal(s) * 0.05)(B, Sk, Dc)),
            "w_q": _w((lambda *s: _rng.normal(s) * 0.05)(M, H, D) * (M ** -0.5)),
            "w_uk": _w((lambda *s: _rng.normal(s) * 0.05)(Dc, H, D) * (Dc ** -0.5)),
            "w_uv": _w((lambda *s: _rng.normal(s) * 0.05)(Dc, H, D) * (Dc ** -0.5)),
            "w_o": _w((lambda *s: _rng.normal(s) * 0.05)(H, D, M) * ((H * D) ** -0.5)),
        }
    _A_in = _A_setup()

    def _B_setup():
        B, Sq, D = 4, 1, 512
        H, Sk, Dh = 32, 4096, 128
        return {
            "x": _w((lambda *s: _rng.normal(s) * 0.05)(B, Sq, D)),
            "k_cache": _w((lambda *s: _rng.normal(s) * 0.05)(B, H, Sk, Dh)),
            "v_cache": _w((lambda *s: _rng.normal(s) * 0.05)(B, H, Sk, Dh)),
            "wq": _w((lambda *s: _rng.normal(s) * 0.05)(D, H * Dh) * (D ** -0.5)),
            "wo": _w((lambda *s: _rng.normal(s) * 0.05)(H * Dh, D) * ((H * Dh) ** -0.5)),
        }
    _B_in = _B_setup()

    return {
        "A_x": _A_in["x"],
        "A_c_kv": _A_in["c_kv"],
        "A_w_q": _A_in["w_q"],
        "A_w_uk": _A_in["w_uk"],
        "A_w_uv": _A_in["w_uv"],
        "A_w_o": _A_in["w_o"],
        "B_x": _B_in["x"],
        "B_k_cache": _B_in["k_cache"],
        "B_v_cache": _B_in["v_cache"],
        "B_wq": _B_in["wq"],
        "B_wo": _B_in["wo"],
    }

def reference(A_x, A_c_kv, A_w_q, A_w_uk, A_w_uv, A_w_o, B_x, B_k_cache, B_v_cache, B_wq, B_wo):
    def _A_ref(x, c_kv, w_q, w_uk, w_uv, w_o):
        B, Sq, M = x.shape[0], x.shape[1], x.shape[2]
        Sk = c_kv.shape[1]
        H, D = w_q.shape[1], w_q.shape[2]
        q = jnp.einsum("bqm,mhd->bhqd", x, w_q)
        k = jnp.einsum("bkc,chd->bhkd", c_kv, w_uk)
        v = jnp.einsum("bkc,chd->bhkd", c_kv, w_uv)
        scores = jnp.einsum("bhqd,bhkd->bhqk", q, k) * (D ** -0.5)
        off = Sk - Sq
        qi = jnp.arange(Sq)[:, None]
        kj = jnp.arange(Sk)[None, :]
        cmask = kj <= (qi + off)
        scores = jnp.where(cmask[None, None], scores, -1e9)
        p = _softmax(scores, axis=-1)
        ctx = jnp.einsum("bhqk,bhkd->bhqd", p, v)
        return jnp.einsum("bhqd,hdm->bqm", ctx, w_o)

    def _B_ref(x, k_cache, v_cache, wq, wo):
        B, Sq, D = x.shape
        H, Dh = 32, 128
        q = (lambda x, *d: x.transpose(*d))((x @ wq).reshape(B, Sq, H, Dh), 0, 2, 1, 3)
        scores = jnp.einsum("bhqd,bhkd->bhqk", q, k_cache) * (Dh ** -0.5)
        p = _softmax(scores, axis=-1)
        o = jnp.einsum("bhqk,bhkd->bhqd", p, v_cache)
        return (lambda x, *d: x.transpose(*d))(o, 0, 2, 1, 3).reshape(B, Sq, H * Dh) @ wo

    a = _A_ref(A_x, A_c_kv, A_w_q, A_w_uk, A_w_uv, A_w_o)
    b = _B_ref(B_x, B_k_cache, B_v_cache, B_wq, B_wo)
    return jnp.concatenate([a, b], axis=-1)
```

```python
import jax
import jax.numpy as jnp
from jax import lax
import jax.experimental.pallas as pl
import jax.experimental.pallas.tpu as pltpu

F32 = jnp.float32
BF16 = jnp.bfloat16
NT = (((1,), (1,)), ((), ()))

NB, NH, SK, HD, DM = 4, 32, 4096, 128, 512
NG = NH // 8
NQ = 4
STEPS = 16
FIRST, LAST = 4, 4 + NH
BLOCK = 64 * 1024
KEYS = BLOCK // (2 * HD)
RING = 8
LEAD = 5
CS = 32
PART = 256
TAIL = 4
SEMS = (2, 5, NB, RING, RING, NH // 2)
HEAD_A, HEAD_B = 32 * 1024, 16 * 1024


def _aligned(x, m):
    return x if isinstance(x, int) else pl.multiple_of(x, m)


def _iota(shape, axis):
    return lax.broadcasted_iota(jnp.int32, shape, axis)


def _kernel(ax_hbm, ckv_hbm, wq_hbm, wuk_hbm, wuv_hbm, wo_hbm, bx_hbm, k_hbm, v_hbm, bwq_hbm, bwo_hbm,
            out_ref,
            ax_v, bx_v, ckv_v, wqv_v, wuk_v, wo_v, bwq_v, bwo_v, k_v, v_v,
            e_v, u_v, acc_v, sa_v, m_v, l_v, c_v, ca_v, oa_v, qb_v, sb_v, pb_v, lb_v, cb_v, ob_v,
            sems):
    scale = HD ** -0.5
    x_sem, w_sem, ckv_sem, k_sem, v_sem, wo_sem = (sems.at[pl.ds(sum(SEMS[:i]), n)] for i, n in enumerate(SEMS))

    def rows(src, dst, head, sem, src_base=0, dst_base=0):
        row_bytes = 2 * src.size // src.shape[0]
        n, a = BLOCK // row_bytes, head // row_bytes

        def copies(q, step):
            i = step & (STEPS - 1)
            starts = (((i - 1) & (STEPS - 1)) * n + n - a, i * n)
            return [pltpu.make_async_copy(src.at[pl.ds(_aligned(src_base + q * STEPS * n + r, a), size)],
                                          dst.at[pl.ds(_aligned(dst_base + q * STEPS * n + r, a), size)], sem(q, step))
                    for r, size in zip(starts, (a, n - a))]
        return copies

    def wide_rows(src, dst, head, sem):
        cols = src.shape[1]
        a = cols * head // BLOCK

        def copies(q, step):
            i = step & (STEPS - 1)
            starts = (((i - 1) & (STEPS - 1)) * 8, i * 8)
            views = [(pl.ds(_aligned(q * STEPS * 8 + r, 8), 8), c)
                     for r, c in zip(starts, (pl.ds(cols - a, a), pl.ds(0, cols - a)))]
            return [pltpu.make_async_copy(src.at[v], dst.at[v], sem(q, step)) for v in views]
        return copies

    def cache(src, dst, sem, h):
        a = HEAD_B // (2 * HD)

        def copies(q, step):
            i, slot = step & (STEPS - 1), step & (RING - 1)
            starts = (((i - 1) & (STEPS - 1)) * KEYS + KEYS - a, i * KEYS)
            return [pltpu.make_async_copy(src.at[pl.ds(_aligned((q * NH + h) * SK + r, a), size)],
                                          dst.at[slot, q, pl.ds(to, size)], sem.at[slot])
                    for r, to, size in zip(starts, (0, a), (a, KEYS - a))]
        return copies

    def wait_all(dst, sem):
        pltpu.make_async_copy(dst, dst, sem).wait()

    def whole(sem):
        return lambda q, step: sem

    def latents(b):
        return rows(ckv_hbm, ckv_v, HEAD_A, whole(ckv_sem.at[b]), b * SK, b * SK)

    wq_sem, wuv_sem, wuk_sem, bwq_sem, bwo_sem = (w_sem.at[i] for i in range(5))
    wo_copies = rows(wo_hbm, wo_v, HEAD_A,
                     lambda q, step: wo_sem.at[(jnp.maximum((step & (STEPS - 1)) - 1, 0) & ~1) + (q >> 1)])

    def start(step, q, *sources):
        for both in zip(*(copies(q, step) for copies in sources)):
            for t, copy in enumerate(both):
                copy.start(priority=t)

    def caches(phase):
        return cache(k_hbm, k_v, k_sem, phase - FIRST), cache(v_hbm, v_v, v_sem, phase - FIRST - 1)

    def start_any(step, first, last):
        phase = step >> 4

        def when(cond, *sources):
            pl.when(cond)(lambda: pl.loop(first, last)(lambda q: start(step, q, *sources)))

        when(phase == 0, rows(wq_hbm, wqv_v, HEAD_A, whole(wq_sem)), wide_rows(bwq_hbm, bwq_v, HEAD_B, whole(bwq_sem)))
        when(phase == 1, rows(wuk_hbm, wuk_v, HEAD_A, whole(wuk_sem)),
             rows(wuv_hbm, wqv_v, HEAD_A, whole(wuv_sem), 0, DM))
        when((phase == 2) | (phase == 3), latents(2 * phase - 4), latents(2 * phase - 3))
        when(phase == FIRST, cache(k_hbm, k_v, k_sem, 0), rows(bwo_hbm, bwo_v, HEAD_B, whole(bwo_sem)))
        when(phase == FIRST + 1, *caches(FIRST + 1))
        when(phase == LAST, cache(v_hbm, v_v, v_sem, NH - 1), wo_copies)

    def same_head(x):
        return jnp.where((_iota(x.shape, 0) & 7) == (_iota(x.shape, 1) & 7), x, 0.0).astype(BF16)

    def a_setup(r):
        shape = (HD, CS * 8)
        e_v[r] = jnp.where(_iota(shape, 0) == r * CS + (_iota(shape, 1) >> 3), 1.0, 0.0).astype(BF16)

    def weight_tile(ref, t, g):
        return ref[pl.ds(t * CS, CS), g].reshape(CS * 8, HD)

    def a_project(t, base):
        u = u_v[t >> 2].reshape(NB * NH, HD).astype(BF16)
        u = same_head(jnp.dot(u, e_v[t & 3], preferred_element_type=F32))
        for g in range(NG):
            w = weight_tile(wqv_v, base + t, g)
            acc_v[g] += jnp.dot(u[g * NB * 8:(g + 1) * NB * 8], w, preferred_element_type=F32)

    def a_absorb(t):
        r = [lax.dot_general(acc_v[g].astype(BF16), weight_tile(wuk_v, t, g), NT, preferred_element_type=F32)
             for g in range(NG)]
        u = lax.dot_general(same_head(jnp.concatenate(r, axis=0)), e_v[t & 3], NT, preferred_element_type=F32)
        u = u.reshape(NG, NB, 8, HD)
        u_v[t >> 2] = jnp.where(_iota(u.shape, 3) // CS == (t & 3), u, u_v[t >> 2])

    def a_attention(b, j):
        parts = SK // PART
        part = j & (parts - 1)
        keys = pl.ds(_aligned(b * SK + part * PART, PART), PART)

        @pl.when(j == 0)
        def _():
            wait_all(ckv_v.at[pl.ds(_aligned(b * SK, SK), SK)], ckv_sem.at[b])
            m_v[...] = jnp.full(m_v.shape, -jnp.inf, F32)

        @pl.when(j < parts)
        def _():
            q = jnp.concatenate([u_v[k, :, b].reshape(NH, HD) for k in range(DM // HD)], axis=1).astype(BF16)
            s = lax.dot_general(q, ckv_v[keys, :], NT, preferred_element_type=F32) * scale
            sa_v[part] = s
            m = m_v[...]
            for k in range(PART // HD):
                m = jnp.maximum(m, s[:, k * HD:(k + 1) * HD])
            m_v[...] = m

        @pl.when(j == parts)
        def _():
            m_v[...] = jnp.broadcast_to(jnp.max(m_v[...], axis=-1, keepdims=True), m_v.shape)
            l_v[...] = jnp.zeros(l_v.shape, F32)
            c_v[...] = jnp.zeros(c_v.shape, F32)

        @pl.when(j >= parts)
        def _():
            p = [jnp.exp(sa_v[part, :, k * HD:(k + 1) * HD] - m_v[...]) for k in range(PART // HD)]
            l_v[...] += sum(p[1:], p[0])
            c_v[...] += jnp.dot(jnp.concatenate(p, axis=1).astype(BF16), ckv_v[keys, :], preferred_element_type=F32)

        @pl.when(j == 2 * parts - 1)
        def _():
            c = c_v[...] / jnp.sum(l_v[...], axis=-1, keepdims=True)
            for k in range(DM // HD):
                u_v[k, :, b] = c[:, k * HD:(k + 1) * HD].reshape(NG, 8, HD)

    def project(ctx, w_ref, h):
        w = w_ref[pl.ds(_aligned(h * HD, HD), HD), :]
        return jnp.dot(ctx.astype(BF16), w, preferred_element_type=F32)

    def a_output(h):
        return project(ca_v[pl.ds(_aligned(8 * h, 8), 8), :], wo_v, h)

    def b_queries(i):
        x = bx_v[...].astype(F32)
        x = jnp.concatenate([x, x], axis=0).astype(BF16)
        q = jnp.dot(x, bwq_v[:, pl.ds(_aligned(i * 2 * HD, 2 * HD), 2 * HD)], preferred_element_type=F32)
        qb_v[2 * i] = q[:, :HD]
        qb_v[2 * i + 1] = q[:, HD:]

    def batch_row(b, x, other):
        return jnp.where(_iota(x.shape, 0) == b, x, other)

    def b_scores(h, i, slot, between=lambda b: None):
        q, s = qb_v[h].astype(BF16), 0.0
        for b in range(NB):
            between(b)
            s = batch_row(b, lax.dot_general(q, k_v[slot, b], NT, preferred_element_type=F32), s)
        sb_v[i] = s * scale

    def b_context(i, slot, between=lambda b: None):
        p, c = pb_v[i].astype(BF16), 0.0
        for b in range(NB):
            between(b)
            c = batch_row(b, jnp.dot(p, v_v[slot, b], preferred_element_type=F32), c)
        cb_v[...] += c

    def b_softmax():
        s = sb_v[...]
        p = jnp.exp(s - jnp.max(jnp.max(s, axis=0), axis=-1, keepdims=True))
        pb_v[...] = p
        lb_v[...] = jnp.sum(jnp.sum(p, axis=0), axis=-1, keepdims=True)
        cb_v[...] = jnp.zeros(cb_v.shape, F32)

    x_copies = [pltpu.make_async_copy(ax_hbm, ax_v, x_sem.at[0]), pltpu.make_async_copy(bx_hbm, bx_v, x_sem.at[1])]
    steps = (LAST + 1) * STEPS
    main = (FIRST + 1) * STEPS
    absorb = main + STEPS
    attention = absorb + STEPS
    values = attention + NB * 2 * SK // PART
    values_done = values + STEPS

    def a_step(g):
        i = g & (STEPS - 1)

        @pl.when((g >= attention) & (g < values))
        def _():
            tiles = 2 * SK // PART
            j = jnp.maximum(g, attention) - attention
            a_attention(j >> (tiles.bit_length() - 1), j & (tiles - 1))

        @pl.when((g < absorb) | ((g >= values) & (g < values_done)))
        def _():
            which = (g >= values).astype(jnp.int32)

            @pl.when(i == 0)
            def _():
                wait_all(wqv_v.at[pl.ds(which * DM, DM)], w_sem.at[which])
                acc_v[...] = jnp.zeros(acc_v.shape, F32)

            a_project(i, which * (DM // CS))

        @pl.when((g >= absorb) & (g < attention))
        def _():
            pl.when(i == 0)(lambda: wait_all(wuk_v, wuk_sem))
            a_absorb(i)

        @pl.when(g == values_done)
        def _():
            @pl.loop(0, NG)
            def _(k):
                shape = (8 * 8, NB * 8)
                r, c = _iota(shape, 0), _iota(shape, 1)
                hit = jnp.where((r & 7) * 8 + (r >> 3) == c, 1.0, 0.0).astype(BF16)
                ctx = jnp.dot(hit, acc_v[k].astype(BF16), preferred_element_type=F32)
                ca_v[pl.ds(_aligned(k * 64, 64), 64), :] = ctx

    def a_tail(u, _):
        k, q = u >> 1, (u & 1) * 2

        @pl.loop(jnp.where(k == 0, 0, 2 * k + 1), jnp.minimum(2 * k + 3, STEPS))
        def _(i):
            for copy in wo_copies(q, i) + wo_copies(q + 1, i):
                copy.wait()

        oa_v[...] += a_output(q * (NH // NQ) + k) + a_output((q + 1) * (NH // NQ) + k)

    def b_output(phase):
        ob_v[...] += project(cb_v[...] / lb_v[...], bwo_v, phase - FIRST - 1)

    def main_step(n, _):
        g = n - LEAD
        phase, i, slot = g >> 4, g & (STEPS - 1), g & (RING - 1)
        wait_all(k_v.at[slot], k_sem.at[slot])
        wait_all(v_v.at[slot], v_sem.at[slot])
        b_scores(phase - FIRST, i, slot, lambda b: None if b % 2 else start(n, b // 2, *caches(n >> 4)))
        b_context(i, slot, lambda b: None if b % 2 else start(n, 2 + b // 2, *caches(n >> 4)))

        @pl.when(i == STEPS - 1)
        def _():
            b_output(phase)
            b_softmax()

        pl.when(g <= values_done)(lambda: a_step(g))

    def edge_compute(g, second):
        phase, i, slot = g >> 4, g & (STEPS - 1), g & (RING - 1)
        scores, context = (phase >= FIRST) & (phase < LAST), phase > FIRST

        @pl.when(~second & scores)
        def _():
            wait_all(k_v.at[slot], k_sem.at[slot])
            b_scores(phase - FIRST, i, slot)

        @pl.when(second & context)
        def _():
            wait_all(v_v.at[slot], v_sem.at[slot])
            b_context(i, slot)

        @pl.when(second & (i == STEPS - 1))
        def _():
            pl.when(context)(lambda: b_output(phase))
            pl.when(scores)(b_softmax)

        @pl.when(second & (phase == LAST) & (i >= TAIL))
        def _():
            @pl.when(i == STEPS - 1)
            def _():
                out_ref[:, pl.ds(DM, DM)] = ob_v[pl.ds(0, NB), :].astype(out_ref.dtype)

            lax.fori_loop(i - TAIL, jnp.where(i == STEPS - 1, STEPS, i - TAIL + 1), a_tail, None)

        @pl.when(second & (g < HD // CS))
        def _():
            a_setup(g)

            @pl.when(g == 0)
            def _():
                for copy in x_copies:
                    copy.start()
                oa_v[...] = jnp.zeros(oa_v.shape, F32)
                ob_v[...] = jnp.zeros(ob_v.shape, F32)

        @pl.when(second & (phase == FIRST - 1))
        def _():
            @pl.when(i == 0)
            def _():
                for copy in x_copies:
                    copy.wait()
                wait_all(bwq_v, bwq_sem)
                x = ax_v[...].astype(F32)

                @pl.loop(0, NG)
                def _(group):
                    for b in range(NB):
                        for k in range(DM // HD):
                            u_v[k, group, b] = jnp.broadcast_to(x[b:b + 1, k * HD:(k + 1) * HD], (8, HD))

            b_queries(i)

    def edge_step(j, _):
        n, half = j >> 1, j & 1
        start_any(n, 2 * half, 2 * half + 2)
        pl.when(n >= LEAD)(lambda: edge_compute(jnp.maximum(n, LEAD) - LEAD, half == 1))

    @pl.loop(0, 2)
    def _(k):
        lax.fori_loop(2 * k * LAST * STEPS, 2 * (jnp.where(k == 0, main, steps) + LEAD), edge_step, None)

        @pl.when(k == 0)
        def _():
            wait_all(bwo_v, bwo_sem)
            lax.fori_loop(main + LEAD, LAST * STEPS, main_step, None)

    out_ref[:, pl.ds(0, DM)] = oa_v[pl.ds(0, NB), :].astype(out_ref.dtype)


@jax.jit
def pallas_concat_heads__compressed_kv_cla__mha_block_cached__decode_kernel(
    A_x: jax.Array,
    A_c_kv: jax.Array,
    A_w_q: jax.Array,
    A_w_uk: jax.Array,
    A_w_uv: jax.Array,
    A_w_o: jax.Array,
    B_x: jax.Array,
    B_k_cache: jax.Array,
    B_v_cache: jax.Array,
    B_wq: jax.Array,
    B_wo: jax.Array,
):
    assert A_x.shape == (NB, 1, DM) and A_c_kv.shape == (NB, SK, DM) and A_w_q.shape == (DM, NH, HD)
    assert B_x.shape == (NB, 1, DM) and B_k_cache.shape == (NB, NH, SK, HD)
    scratch = [
        pltpu.VMEM((NB, DM), BF16),
        pltpu.VMEM((NB, DM), BF16),
        pltpu.VMEM((NB * SK, DM), BF16),
        pltpu.VMEM((2 * DM, NG, 8, HD), BF16),
        pltpu.VMEM((DM, NG, 8, HD), BF16),
        pltpu.VMEM((NH * HD, DM), BF16),
        pltpu.VMEM((DM, NH * HD), BF16),
        pltpu.VMEM((NH * HD, DM), BF16),
        pltpu.VMEM((RING, NB, KEYS, HD), BF16),
        pltpu.VMEM((RING, NB, KEYS, HD), BF16),
        pltpu.VMEM((HD // CS, HD, CS * 8), BF16),
        pltpu.VMEM((DM // HD, NG, NB, 8, HD), F32),
        pltpu.VMEM((NG, NB * 8, HD), F32),
        pltpu.VMEM((SK // PART, NH, PART), F32),
        pltpu.VMEM((NH, HD), F32),
        pltpu.VMEM((NH, HD), F32),
        pltpu.VMEM((NH, DM), F32),
        pltpu.VMEM((8 * NH, HD), F32),
        pltpu.VMEM((8, DM), F32),
        pltpu.VMEM((NH, 8, HD), F32),
        pltpu.VMEM((STEPS, 8, KEYS), F32),
        pltpu.VMEM((STEPS, 8, KEYS), F32),
        pltpu.VMEM((8, 1), F32),
        pltpu.VMEM((8, HD), F32),
        pltpu.VMEM((8, DM), F32),
        pltpu.SemaphoreType.DMA((sum(SEMS),)),
    ]
    out = pl.pallas_call(
        _kernel,
        out_shape=jax.ShapeDtypeStruct((NB, 2 * DM), A_x.dtype),
        in_specs=[pl.BlockSpec(memory_space=pl.ANY)] * 11,
        out_specs=pl.BlockSpec(memory_space=pltpu.VMEM),
        scratch_shapes=scratch,
        compiler_params=pltpu.CompilerParams(
            vmem_limit_bytes=100 * 1024 * 1024, disable_bounds_checks=True, disable_semaphore_checks=True),
    )(
        A_x.reshape(NB, DM),
        A_c_kv.reshape(NB * SK, DM),
        A_w_q.reshape(DM, NG, 8, HD),
        A_w_uk.reshape(DM, NG, 8, HD),
        A_w_uv.reshape(DM, NG, 8, HD),
        A_w_o.reshape(NH * HD, DM),
        B_x.reshape(NB, DM),
        B_k_cache.reshape(NB * NH * SK, HD),
        B_v_cache.reshape(NB * NH * SK, HD),
        B_wq,
        B_wo,
    )
    return out.reshape(NB, 1, 2 * DM)
```

```python
import functools

import jax
import jax.numpy as jnp
from jax import lax
import jax.experimental.pallas as pl
import jax.experimental.pallas.tpu as pltpu

F32 = jnp.float32
BF16 = jnp.bfloat16
NT = (((1,), (1,)), ((), ()))

NB, NH, SK, HD, DM = 4, 32, 4096, 128, 512
NG = NH // 8
NQ = 4
STEPS = 16
FIRST, LAST = 4, 4 + NH
BLOCK = 64 * 1024
KEYS = BLOCK // (2 * HD)
QUARTER = NH * HD // NQ
RING = 8
LEAD = 6
FILL = 8
TAIL = 5
CS = 32
PART = 256
SPLIT_A, SPLIT_B = 32 * 1024, 16 * 1024
SEMS = (2, 5, NB, RING, RING, STEPS // 2 + 2)


def _aligned(x, m):
    return x if isinstance(x, int) else pl.multiple_of(x, m)


def _iota(shape, axis):
    return lax.broadcasted_iota(jnp.int32, shape, axis)


def _wait_all(dst, sem):
    pltpu.make_async_copy(dst, dst, sem).wait()


def _body(ax_hbm, ckv_hbm, wq_hbm, wuk_hbm, wuv_hbm, wo_hbm, bx_hbm, k_hbm, v_hbm, bwq_hbm, bwo_hbm,
          out_ref,
          ax_v, bx_v, ckv_v, wqv_v, wuk_v, wo_v, bwq_v, bwo_v, k_v, v_v,
          e_v, u_v, acc_v, sa_v, m_v, l_v, c_v, ca_v, oa_v, qb_v, sb_v, pb_v, lb_v, cb_v, ob_v,
          sems):
    scale = HD ** -0.5
    x_sem, w_sem, ckv_sem, k_sem, v_sem, wo_sem = (sems.at[pl.ds(sum(SEMS[:i]), n)] for i, n in enumerate(SEMS))
    wq_sem, wuv_sem, wuk_sem, bwq_sem, bwo_sem = (w_sem.at[i] for i in range(5))

    def block(i, size, split):
        return (((i - 1) & (STEPS - 1)) * size + size - split, split), ((i & (STEPS - 1)) * size, size - split)

    def rows(src, dst, split, sem, src_base=0, dst_base=0):
        row_bytes = 2 * src.size // src.shape[0]
        size, split = BLOCK // row_bytes, split // row_bytes

        def copies(q, step):
            return [pltpu.make_async_copy(src.at[pl.ds(_aligned(src_base + q * STEPS * size + r, split), n)],
                                          dst.at[pl.ds(_aligned(dst_base + q * STEPS * size + r, split), n)], sem)
                    for r, n in block(step, size, split)]
        return copies

    def bwq_copies(q, step):
        split = NH * HD * SPLIT_B // BLOCK
        views = [(pl.ds(_aligned((q * STEPS + (i & (STEPS - 1))) * 8, 8), 8), cols)
                 for i, cols in ((step - 1, pl.ds(NH * HD - split, split)), (step, pl.ds(0, NH * HD - split)))]
        return [pltpu.make_async_copy(bwq_hbm.at[view], bwq_v.at[view], bwq_sem) for view in views]

    def wo_copies(q, step):
        i, size, split = step & (STEPS - 1), BLOCK // (2 * DM), SPLIT_A // (2 * DM)
        sem = wo_sem.at[((i + 1) >> 1) + jnp.where(i == STEPS - 1, q >> 1, 0)]
        return [pltpu.make_async_copy(wo_hbm.at[pl.ds(_aligned(q * QUARTER + r, split), n)],
                                      wo_v.at[q, pl.ds(_aligned(r, split), n)], sem)
                for r, n in block(step, size, split)]

    def cache(src, dst, sem, h):
        split = SPLIT_B // (2 * HD)

        def copies(q, step):
            slot = step & (RING - 1)
            return [pltpu.make_async_copy(src.at[pl.ds(_aligned((q * NH + h) * SK + r, split), n)],
                                          dst.at[slot, q, pl.ds(to, n)], sem.at[slot])
                    for (r, n), to in zip(block(9 * step + 2 * q, KEYS, split), (0, split))]
        return copies

    def caches(phase):
        return cache(k_hbm, k_v, k_sem, phase - FIRST), cache(v_hbm, v_v, v_sem, phase - FIRST - 1)

    def latents(b):
        return rows(ckv_hbm, ckv_v, SPLIT_A, ckv_sem.at[b], b * SK, b * SK)

    queries = rows(wq_hbm, wqv_v, SPLIT_A, wq_sem), bwq_copies

    def start(step, q, sources, priorities=(0, 1)):
        for pair in zip(*(copies(q, step) for copies in sources)):
            for copy, priority in zip(pair, priorities):
                copy.start(priority=priority)

    def start_half(step, half):
        phase = step >> 4

        def when(cond, *sources):
            pl.when(cond)(lambda: pl.loop(2 * half, 2 * half + 2)(lambda q: start(step, q, sources)))

        when(phase == 0, *queries)
        when(phase == 1, rows(wuk_hbm, wuk_v, SPLIT_A, wuk_sem), rows(wuv_hbm, wqv_v, SPLIT_A, wuv_sem, 0, DM))
        when((phase == 2) | (phase == 3), latents(2 * phase - 4), latents(2 * phase - 3))
        when(phase == FIRST, cache(k_hbm, k_v, k_sem, 0), rows(bwo_hbm, bwo_v, SPLIT_B, bwo_sem))
        when(phase == FIRST + 1, *caches(FIRST + 1))
        when(phase == LAST, cache(v_hbm, v_v, v_sem, NH - 1), wo_copies)

    def a_setup(r):
        shape = (HD, CS * 8)
        e_v[r] = jnp.where(_iota(shape, 0) == r * CS + (_iota(shape, 1) >> 3), 1.0, 0.0).astype(BF16)

    def a_input():
        x = ax_v[...].astype(F32)

        @pl.loop(0, NG)
        def _(g):
            for b in range(NB):
                for k in range(DM // HD):
                    u_v[k, g, b] = jnp.broadcast_to(x[b:b + 1, k * HD:(k + 1) * HD], (8, HD))

    def same_head(x):
        return jnp.where((_iota(x.shape, 0) & 7) == (_iota(x.shape, 1) & 7), x, 0.0).astype(BF16)

    def weight_tile(ref, t, g):
        return ref[pl.ds(t * CS, CS), g].reshape(CS * 8, HD)

    def a_project(t, base):
        u = u_v[t >> 2].reshape(NB * NH, HD).astype(BF16)
        u = same_head(jnp.dot(u, e_v[t & 3], preferred_element_type=F32))
        for g in range(NG):
            w = weight_tile(wqv_v, base + t, g)
            acc_v[g] += jnp.dot(u[g * NB * 8:(g + 1) * NB * 8], w, preferred_element_type=F32)

    def a_absorb(t):
        r = [lax.dot_general(acc_v[g].astype(BF16), weight_tile(wuk_v, t, g), NT, preferred_element_type=F32)
             for g in range(NG)]
        u = lax.dot_general(same_head(jnp.concatenate(r, axis=0)), e_v[t & 3], NT, preferred_element_type=F32)
        u = u.reshape(NG, NB, 8, HD)
        u_v[t >> 2] = jnp.where(_iota(u.shape, 3) // CS == (t & 3), u, u_v[t >> 2])

    def a_attention(b, j):
        parts = SK // PART
        part = j & (parts - 1)
        keys = pl.ds(_aligned(b * SK + part * PART, PART), PART)

        @pl.when(j == 0)
        def _():
            _wait_all(ckv_v.at[pl.ds(_aligned(b * SK, SK), SK)], ckv_sem.at[b])
            m_v[...] = jnp.full(m_v.shape, -jnp.inf, F32)

        @pl.when(j < parts)
        def _():
            q = jnp.concatenate([u_v[k, :, b].reshape(NH, HD) for k in range(DM // HD)], axis=1).astype(BF16)
            s = lax.dot_general(q, ckv_v[keys, :], NT, preferred_element_type=F32) * scale
            sa_v[part] = s
            m = m_v[...]
            for k in range(PART // HD):
                m = jnp.maximum(m, s[:, k * HD:(k + 1) * HD])
            m_v[...] = m

        @pl.when(j == parts)
        def _():
            m_v[...] = jnp.broadcast_to(jnp.max(m_v[...], axis=-1, keepdims=True), m_v.shape)
            l_v[...] = jnp.zeros(l_v.shape, F32)
            c_v[...] = jnp.zeros(c_v.shape, F32)

        @pl.when(j >= parts)
        def _():
            p = [jnp.exp(sa_v[part, :, k * HD:(k + 1) * HD] - m_v[...]) for k in range(PART // HD)]
            l_v[...] += sum(p[1:], p[0])
            c_v[...] += jnp.dot(jnp.concatenate(p, axis=1).astype(BF16), ckv_v[keys, :], preferred_element_type=F32)

        @pl.when(j == 2 * parts - 1)
        def _():
            c = c_v[...] / jnp.sum(l_v[...], axis=-1, keepdims=True)
            for k in range(DM // HD):
                u_v[k, :, b] = c[:, k * HD:(k + 1) * HD].reshape(NG, 8, HD)

    def a_head_major(g):
        shape = (8 * 8, NB * 8)
        r, c = _iota(shape, 0), _iota(shape, 1)
        pick = jnp.where((r & 7) * 8 + (r >> 3) == c, 1.0, 0.0).astype(BF16)
        ca_v[pl.ds(_aligned(g * 64, 64), 64), :] = jnp.dot(pick, acc_v[g].astype(BF16), preferred_element_type=F32)

    def project(ctx, w_ref, h):
        w = w_ref[pl.ds(_aligned(h * HD, HD), HD), :]
        return jnp.dot(ctx.astype(BF16), w, preferred_element_type=F32)

    def a_output(o, k, streams):
        for q in streams:
            o = o + project(ca_v[pl.ds(_aligned(8 * (q * NH // NQ + k), 8), 8), :], wo_v.at[q], k)
        return o

    def b_queries(i):
        x = bx_v[...].astype(F32)
        x = jnp.concatenate([x, x], axis=0).astype(BF16)
        q = jnp.dot(x, bwq_v[:, pl.ds(_aligned(i * 2 * HD, 2 * HD), 2 * HD)], preferred_element_type=F32)
        qb_v[2 * i] = q[:, :HD]
        qb_v[2 * i + 1] = q[:, HD:]

    def per_batch(product, between):
        rows = 0.0
        for b in range(NB):
            between(b)
            x = product(b)
            rows = jnp.where(_iota(x.shape, 0) == b, x, rows)
        return rows

    def b_scores(h, i, slot, between=lambda b: None):
        q = qb_v[h].astype(BF16)
        s = per_batch(lambda b: lax.dot_general(q, k_v[slot, b], NT, preferred_element_type=F32), between)
        sb_v[i] = s * scale

    def b_softmax():
        s = sb_v[...]
        p = jnp.exp(s - jnp.max(jnp.max(s, axis=0), axis=-1, keepdims=True))
        pb_v[...] = p
        lb_v[...] = jnp.sum(jnp.sum(p, axis=0), axis=-1, keepdims=True)
        cb_v[...] = jnp.zeros(cb_v.shape, F32)

    def b_context(i, slot, between=lambda b: None):
        p = pb_v[i].astype(BF16)
        cb_v[...] += per_batch(lambda b: jnp.dot(p, v_v[slot, b], preferred_element_type=F32), between)

    def b_output(h):
        ob_v[...] += project(cb_v[...] / lb_v[...], bwo_v, h)

    main = (FIRST + 1) * STEPS
    absorb = main + STEPS
    attention = absorb + STEPS
    values = attention + NB * 2 * SK // PART
    values_done = values + STEPS

    def a_step(g):
        i = g & (STEPS - 1)

        @pl.when((g >= attention) & (g < values))
        def _():
            tiles = 2 * SK // PART
            j = jnp.maximum(g, attention) - attention
            a_attention(j >> (tiles.bit_length() - 1), j & (tiles - 1))

        @pl.when((g < absorb) | ((g >= values) & (g < values_done)))
        def _():
            which = (g >= values).astype(jnp.int32)

            @pl.when(i == 0)
            def _():
                _wait_all(wqv_v.at[pl.ds(which * DM, DM)], w_sem.at[which])
                acc_v[...] = jnp.zeros(acc_v.shape, F32)

            a_project(i, which * (DM // CS))

        @pl.when((g >= absorb) & (g < attention))
        def _():
            pl.when(i == 0)(lambda: _wait_all(wuk_v, wuk_sem))
            a_absorb(i)

        pl.when(g == values_done)(lambda: pl.loop(0, NG)(a_head_major))

    def main_step(n):
        g = n - LEAD
        h, i, slot = (g >> 4) - FIRST, g & (STEPS - 1), g & (RING - 1)
        _wait_all(k_v.at[slot], k_sem.at[slot])
        _wait_all(v_v.at[slot], v_sem.at[slot])
        b_scores(h, i, slot, lambda b: None if b % 2 else start(n, b // 2, caches(n >> 4)))
        b_context(i, slot, lambda b: None if b % 2 else start(n, 2 + b // 2, caches(n >> 4)))

        @pl.when(i == STEPS - 1)
        def _():
            b_output(h - 1)
            b_softmax()

        pl.when(g <= values_done)(lambda: a_step(g))

    wo_size, wo_split = BLOCK // (2 * DM), SPLIT_A // (2 * DM)
    x_copies = [pltpu.make_async_copy(ax_hbm, ax_v, x_sem.at[0]), pltpu.make_async_copy(bx_hbm, bx_v, x_sem.at[1])]

    def edge_compute(g, second):
        phase, i, slot = g >> 4, g & (STEPS - 1), g & (RING - 1)
        scores, context = (phase >= FIRST) & (phase < LAST), phase > FIRST

        @pl.when(~second & scores)
        def _():
            _wait_all(k_v.at[slot], k_sem.at[slot])
            b_scores(phase - FIRST, i, slot)

        @pl.when(second & context)
        def _():
            _wait_all(v_v.at[slot], v_sem.at[slot])
            b_context(i, slot)

        @pl.when(second & (i == STEPS - 1))
        def _():
            pl.when(context)(lambda: b_output(phase - FIRST - 1))
            pl.when(scores)(b_softmax)

        @pl.when(second & (phase == LAST) & (i >= TAIL) & ((i & 1) == 1))
        def _():
            @pl.when(i == TAIL)
            def _():
                @pl.loop(0, NQ)
                def _(q):
                    for copy in wo_copies(q, 0):
                        copy.wait()

            @pl.loop((i - TAIL) >> 1, jnp.where(i == STEPS - 1, STEPS // 2 - 1, ((i - TAIL) >> 1) + 1))
            def _(k):
                _wait_all(wo_v.at[:, pl.ds(_aligned(k * HD + wo_size - wo_split, wo_split), HD)], wo_sem.at[k + 1])
                oa_v[...] = a_output(oa_v[...], k, range(NQ))

        @pl.when(second & (g < HD // CS))
        def _():
            a_setup(g)

            @pl.when(g == 0)
            def _():
                for copy in x_copies:
                    copy.start()
                oa_v[...] = jnp.zeros(oa_v.shape, F32)
                ob_v[...] = jnp.zeros(ob_v.shape, F32)

        @pl.when(second & (phase == FIRST - 1))
        def _():
            @pl.when(i == 0)
            def _():
                for copy in x_copies:
                    copy.wait()
                _wait_all(bwq_v, bwq_sem)
                a_input()

            b_queries(i)

    def edge_step(j):
        n, half = j >> 1, j & 1
        start_half(n, half)
        pl.when(n >= LEAD)(lambda: edge_compute(jnp.maximum(n, LEAD) - LEAD, half == 1))

    pl.loop(0, FILL)(lambda j: start(j >> 2, j & (NQ - 1), queries, (1, 1)))

    @pl.loop(0, 2)
    def _(after):
        end = jnp.where(after == 0, main, (LAST + 1) * STEPS) + LEAD
        pl.loop(jnp.where(after == 0, FILL // 2, 2 * LAST * STEPS), 2 * end)(edge_step)

        @pl.when(after == 0)
        def _():
            _wait_all(bwo_v, bwo_sem)
            pl.loop(main + LEAD, LAST * STEPS)(main_step)

    out_ref[:, pl.ds(DM, DM)] = ob_v[pl.ds(0, NB), :].astype(out_ref.dtype)
    o = oa_v[...]
    for half in range(2):
        _wait_all(wo_v.at[pl.ds(2 * half, 2), pl.ds(QUARTER - wo_size - wo_split, wo_size)],
                  wo_sem.at[STEPS // 2 + half])
        o = a_output(o, STEPS // 2 - 1, (2 * half, 2 * half + 1))
    out_ref[:, pl.ds(0, DM)] = o[:NB].astype(out_ref.dtype)


def _kernel(*refs):
    pl.run_scoped(functools.partial(_body, *refs), pltpu.SemaphoreType.DMA((sum(SEMS),)))


@jax.jit
def pallas_concat_heads__compressed_kv_cla__mha_block_cached__decode_kernel(
    A_x: jax.Array,
    A_c_kv: jax.Array,
    A_w_q: jax.Array,
    A_w_uk: jax.Array,
    A_w_uv: jax.Array,
    A_w_o: jax.Array,
    B_x: jax.Array,
    B_k_cache: jax.Array,
    B_v_cache: jax.Array,
    B_wq: jax.Array,
    B_wo: jax.Array,
):
    assert A_x.shape == (NB, 1, DM) and A_c_kv.shape == (NB, SK, DM) and A_w_q.shape == (DM, NH, HD)
    assert B_x.shape == (NB, 1, DM) and B_k_cache.shape == (NB, NH, SK, HD)
    scratch = [
        pltpu.VMEM((NB, DM), BF16),
        pltpu.VMEM((NB, DM), BF16),
        pltpu.VMEM((NB * SK, DM), BF16),
        pltpu.VMEM((2 * DM, NG, 8, HD), BF16),
        pltpu.VMEM((DM, NG, 8, HD), BF16),
        pltpu.VMEM((NQ, QUARTER, DM), BF16),
        pltpu.VMEM((DM, NH * HD), BF16),
        pltpu.VMEM((NH * HD, DM), BF16),
        pltpu.VMEM((RING, NB, KEYS, HD), BF16),
        pltpu.VMEM((RING, NB, KEYS, HD), BF16),
        pltpu.VMEM((HD // CS, HD, CS * 8), BF16),
        pltpu.VMEM((DM // HD, NG, NB, 8, HD), F32),
        pltpu.VMEM((NG, NB * 8, HD), F32),
        pltpu.VMEM((SK // PART, NH, PART), F32),
        pltpu.VMEM((NH, HD), F32),
        pltpu.VMEM((NH, HD), F32),
        pltpu.VMEM((NH, DM), F32),
        pltpu.VMEM((8 * NH, HD), F32),
        pltpu.VMEM((8, DM), F32),
        pltpu.VMEM((NH, 8, HD), F32),
        pltpu.VMEM((STEPS, 8, KEYS), F32),
        pltpu.VMEM((STEPS, 8, KEYS), F32),
        pltpu.VMEM((8, 1), F32),
        pltpu.VMEM((8, HD), F32),
        pltpu.VMEM((8, DM), F32),
    ]
    out = pl.pallas_call(
        _kernel,
        out_shape=jax.ShapeDtypeStruct((NB, 2 * DM), A_x.dtype),
        in_specs=[pl.BlockSpec(memory_space=pl.ANY)] * 11,
        out_specs=pl.BlockSpec(memory_space=pltpu.VMEM),
        scratch_shapes=scratch,
        compiler_params=pltpu.CompilerParams(vmem_limit_bytes=100 * 1024 * 1024),
    )(
        A_x.reshape(NB, DM),
        A_c_kv.reshape(NB * SK, DM),
        A_w_q.reshape(DM, NG, 8, HD),
        A_w_uk.reshape(DM, NG, 8, HD),
        A_w_uv.reshape(DM, NG, 8, HD),
        A_w_o.reshape(NH * HD, DM),
        B_x.reshape(NB, DM),
        B_k_cache.reshape(NB * NH * SK, HD),
        B_v_cache.reshape(NB * NH * SK, HD),
        B_wq,
        B_wo,
    )
    return out.reshape(NB, 1, 2 * DM)
```
